```python
import jax
import jax.numpy as jnp

def _softmax(x, axis=-1):
    return jax.nn.softmax(x, axis=axis)
def _gelu(x):
    return jax.nn.gelu(x, approximate=True)
def _silu(x):
    return jax.nn.silu(x)
def _sigmoid(x):
    return jax.nn.sigmoid(x)
def _layernorm(x, axis=-1, eps=1e-5):
    m = jnp.mean(x, axis=axis, keepdims=True)
    v = jnp.var(x, axis=axis, keepdims=True)
    return (x - m) / jnp.sqrt(v + eps)
def _scatter_add(tgt, idx, src, axis=0):
    return tgt.at[idx].add(src)
def _segment_sum(src, seg, n):
    return jax.ops.segment_sum(src, seg, n)
class _Rng:
    def __init__(self, key):
        self._k = key
    def _next(self):
        self._k, sub = jax.random.split(self._k)
        return sub
    def normal(self, shape):
        return jax.random.normal(self._next(), shape, dtype=jnp.bfloat16)
    def randint(self, lo, hi, shape):
        return jax.random.randint(self._next(), shape, lo, hi, dtype=jnp.int32)
    def uniform(self, shape, lo=0.0, hi=1.0):
        return jax.random.uniform(self._next(), shape, jnp.bfloat16, lo, hi)
    def permutation(self, n):
        return jax.random.permutation(self._next(), n)


kernel_name = 'interleave_layers__sliding_block_cached__dense_activation_gelu__decode'

def setup_inputs():
    _rng = _Rng(jax.random.key(int.from_bytes(__import__("os").urandom(4), "little")))
    _w = (lambda a: (lambda t: t.astype(jnp.bfloat16) if jnp.issubdtype(t.dtype, jnp.floating) else t)(jnp.asarray(a)))
    def _A_setup():
        B, Sq, D = 1, 1, 640
        Hq, Hkv, Sk, Dh = 32, 32, 32768, 192
        assert Hq % Hkv == 0, (Hq, Hkv)
        return {
            "x": _w((lambda *s: _rng.normal(s) * 0.05)(B, Sq, D)),
            "k_cache": _w((lambda *s: _rng.normal(s) * 0.05)(B, Hkv, Sk, Dh)),
            "v_cache": _w((lambda *s: _rng.normal(s) * 0.05)(B, Hkv, Sk, Dh)),
            "wq": _w((lambda *s: _rng.normal(s) * 0.05)(D, Hq * Dh) * (D ** -0.5)),
            "wo": _w((lambda *s: _rng.normal(s) * 0.05)(Hq * Dh, D) * ((Hq * Dh) ** -0.5)),
        }
    _A_in = _A_setup()

    def _B_setup():
        B, S, D, F = 1, 1, 640, 1536
        return {
            "x": _w((lambda *s: _rng.normal(s) * 0.05)(B, S, D)),
            "w1": _w((lambda *s: _rng.normal(s) * 0.05)(D, F) * (D ** -0.5)),
            "b1": _w((lambda *s: _rng.normal(s) * 0.05)(F) * 0.01),
            "w2": _w((lambda *s: _rng.normal(s) * 0.05)(F, D) * (F ** -0.5)),
            "b2": _w((lambda *s: _rng.normal(s) * 0.05)(D) * 0.01),
        }
    _B_in = _B_setup()

    return {
        "A_x": _A_in["x"],
        "A_k_cache": _A_in["k_cache"],
        "A_v_cache": _A_in["v_cache"],
        "A_wq": _A_in["wq"],
        "A_wo": _A_in["wo"],
        "B_x": _B_in["x"],
        "B_w1": _B_in["w1"],
        "B_b1": _B_in["b1"],
        "B_w2": _B_in["w2"],
        "B_b2": _B_in["b2"],
    }

def reference(A_x, A_k_cache, A_v_cache, A_wq, A_wo, B_x, B_w1, B_b1, B_w2, B_b2):
    def _A_ref(x, k_cache, v_cache, wq, wo):
        B, Sq, D = x.shape
        Hq, Dh = 32, 192
        Hkv, Sk = k_cache.shape[1], k_cache.shape[2]
        W = min(4096, max(256, Sk // 4))
        rep = Hq // Hkv
        q = (lambda x, *d: x.transpose(*d))((x @ wq).reshape(B, Sq, Hq, Dh), 0, 2, 1, 3)
        k = jnp.repeat(k_cache[:, :, Sk - W:, :], rep, axis=1)
        v = jnp.repeat(v_cache[:, :, Sk - W:, :], rep, axis=1)
        scores = jnp.einsum("bhqd,bhkd->bhqk", q, k) * (Dh ** -0.5)
        p = _softmax(scores, axis=-1)
        o = jnp.einsum("bhqk,bhkd->bhqd", p, v)
        return (lambda x, *d: x.transpose(*d))(o, 0, 2, 1, 3).reshape(B, Sq, Hq * Dh) @ wo

    def _B_ref(x, w1, b1, w2, b2):
        h = jnp.einsum("bsd,df->bsf", x, w1) + b1
        h = _gelu(h)
        return jnp.einsum("bsf,fd->bsd", h, w2) + b2

    x = A_x
    x = x + _A_ref(_layernorm(x, axis=-1), A_k_cache, A_v_cache, A_wq, A_wo)
    x = x + _B_ref(_layernorm(x, axis=-1), B_w1, B_b1, B_w2, B_b2)
    x = x + _A_ref(_layernorm(x, axis=-1), A_k_cache, A_v_cache, A_wq, A_wo)
    x = x + _B_ref(_layernorm(x, axis=-1), B_w1, B_b1, B_w2, B_b2)
    return x
```

```python
import jax
import jax.numpy as jnp
from jax import lax
import jax.experimental.pallas as pl
import jax.experimental.pallas.tpu as pltpu

D, F = 640, 1536
H, DH = 32, 192
W = 4096
NP = H // 2
CT = W // 128
NCH = 4
PPC = NP // NCH
N_MXU_PV = 2
RB = 4

BF, F32, U32 = jnp.bfloat16, jnp.float32, jnp.uint32


def _tiles(a):
    r, c = a.shape
    return a.reshape(r // 16, 2, 8, c // 128, 128).transpose(0, 1, 3, 2, 4)


def _kernel(x_hbm, k_hbm, v_hbm, wq_hbm, wo_hbm, w1_hbm, b1_hbm, w2_hbm, b2_hbm, o_ref,
            kb, vb, wqb, wob, w1b, w2b, xb, b1b, b2b, ob, sp, pb, sems):
    ct0 = k_hbm.shape[2] - CT
    ku, vu, wqu, wou, w1u, w2u = (r.bitcast(U32) for r in (kb, vb, wqb, wob, w1b, w2b))

    def copies(src, dst, r0, nr, c0, sem):
        nc = dst.shape[1]
        return [pltpu.make_async_copy(src.at[pl.ds(r0, nr), par, pl.ds(c0, nc)],
                                      dst.at[pl.ds(r0, nr), :, pl.ds(par * 8, 8), :],
                                      sems.at[sem]) for par in range(2)]

    rpc = PPC * 24
    jobs = [copies(wq_hbm, wqb, 0, D // 16, 0, 0)]
    for c in range(NCH):
        jobs.append(copies(k_hbm, kb, c * rpc, rpc, ct0, len(jobs)))
        jobs.append(copies(v_hbm, vb, c * rpc, rpc, ct0, len(jobs)))
    jobs.append(copies(w1_hbm, w1b, 0, D // 16, 0, len(jobs)))
    jobs.append(copies(wo_hbm, wob, 0, 192, 0, len(jobs)))
    jobs.append(copies(wo_hbm, wob, 192, 192, 0, len(jobs)))
    jobs.append(copies(w2_hbm, w2b, 0, F // 16, 0, len(jobs)))
    small = [pltpu.make_async_copy(s, d, sems.at[len(jobs) + i])
             for i, (s, d) in enumerate(((x_hbm, xb), (b1_hbm, b1b), (b2_hbm, b2b)))]

    def start(j):
        for cp in jobs[j]:
            cp.start()

    def finish(j):
        for cp in jobs[j]:
            cp.wait()
        if j + 2 < len(jobs):
            start(j + 2)

    row = lax.broadcasted_iota(jnp.int32, (8, 128), 0)
    lane = lax.broadcasted_iota(jnp.int32, (8, 128), 1)
    even = (row & 1) == 0
    lo64 = lane < 64

    def wtile(ref, r0, n, c):
        return pltpu.bitcast(ref[pl.ds(r0, n), c].reshape(n * 8, 128), BF)

    def dot(a, b):
        return jnp.dot(a, b, preferred_element_type=F32)

    def project(lhs, ref, r0, n, c0, nc):
        return dot(lhs, jnp.concatenate([wtile(ref, r0, n, c0 + c) for c in range(nc)], axis=1))

    def layernorm(x):
        m = jnp.sum(x, axis=-1, keepdims=True) * (1.0 / D)
        xc = x - m
        v = jnp.sum(xc * xc, axis=-1, keepdims=True) * (1.0 / D)
        return (xc / jnp.sqrt(v + 1e-5)).astype(BF)

    def ffn_up(x):
        h = project(layernorm(x), w1u, 0, D // 16, 0, F // 128) + b1b[...].astype(F32).reshape(1, F)
        return jax.nn.gelu(h, approximate=True).astype(BF)

    def ffn_down(x, h):
        return x + (project(h, w2u, 0, F // 16, 0, D // 128) + b2b[...].astype(F32).reshape(1, D))

    def qk(j, xn, slot):
        q = project(xn, wqu, 0, D // 16, j * 3, 3)
        own = (even, even == lo64, ~even)
        lhs = [[jnp.where(own[t] & ((row >> 1) == u), q[:, t * 128:(t + 1) * 128], 0.0).astype(BF)
                for u in range(4)] for t in range(3)]
        for g in range(CT // 4):
            for t in range(3):
                for u in range(4):
                    sp[slot, g, t * 4 + u] = dot(lhs[t][u], wtile(ku, j * 24 + t * 8, 8, g * 4 + u))

    def over_head(x, op):
        x = op(x, pltpu.roll(x, 2, 0))
        return op(x, pltpu.roll(x, 4, 0))

    def tree(xs, op):
        while len(xs) > 1:
            xs = [op(*xs[i:i + 2]) if i + 1 < len(xs) else xs[i] for i in range(0, len(xs), 2)]
        return xs[0]

    def softmax(slot):
        s = [tree([sp[slot, g, i] for i in range(12)], jnp.add) * (DH ** -0.5) for g in range(CT // 4)]
        m = jnp.max(over_head(tree(s, jnp.maximum), jnp.maximum), axis=-1, keepdims=True)
        p = [jnp.exp(x - m) for x in s]
        l = jnp.sum(over_head(tree(p, jnp.add), jnp.add), axis=-1, keepdims=True)
        return p, jnp.broadcast_to(1.0 / l, (8, 128))

    def pv_mxu(j, p, inv):
        acc = None
        for g in range(CT // 4):
            lhs = jnp.concatenate([jnp.where((row >> 1) == u, p[g], 0.0) for u in range(4)], axis=1)
            rhs = jnp.concatenate([wtile(vu, j * 24, 24, g * 4 + u) for u in range(4)], axis=1)
            o = lax.dot_general(lhs.astype(BF), rhs, (((1,), (1,)), ((), ())), preferred_element_type=F32)
            acc = o if acc is None else acc + o
        own = (even, even == lo64, ~even)
        out = []
        for t in range(3):
            o = over_head(acc[:, t * 128:(t + 1) * 128], jnp.add) * inv
            out.append(jnp.where(own[t], o, pltpu.roll(o, 1, 0)))
        return jnp.concatenate(out, axis=1)

    def pv_vpu(j, p, inv, slot):
        for g in range(CT // 4):
            for r in range(8):
                pb[slot, r & 1, g * 4 + (r >> 1)] = jnp.broadcast_to(p[g][r:r + 1, :], (8, 128))
        accs = []
        for r0 in range(0, 24, RB):
            acc = [None] * RB
            for g in range(CT // 4):
                pu = [pb[slot, r0 // 12, g * 4 + u] for u in range(4)]
                pu = [jnp.concatenate([x, x], axis=0) for x in pu]
                for r in range(RB):
                    t = tree([pltpu.bitcast(vu[j * 24 + r0 + r, g * 4 + u], BF).astype(F32) * pu[u]
                              for u in range(4)], jnp.add)
                    acc[r] = t if g == 0 else acc[r] + t
            accs += acc
        other = pltpu.roll(inv, 1, 0)
        own = (even, even == lo64, ~even)
        out = []
        for t in range(3):
            a = jnp.concatenate(accs[t * 8:(t + 1) * 8], axis=0).T
            a = tree([a[i * 8:(i + 1) * 8] for i in range(16)], jnp.add)
            a = over_head(a + pltpu.roll(a, 1, 0), jnp.add)
            out.append(a * jnp.where(own[t], inv, other))
        return jnp.concatenate(out, axis=1)

    def out_proj(j, o):
        return project(o.astype(BF), wou, j * 24, 24, 0, D // 128)

    start(0)
    for cp in small:
        cp.start()
    start(1)
    for cp in small:
        cp.wait()
    x = jnp.broadcast_to(xb[0].astype(F32), (8, D))
    xn = layernorm(x)
    finish(0)

    @pl.loop(0, NP)
    def _(j):
        for c in range(NCH):
            @pl.when(j == c * PPC)
            def _():
                finish(1 + 2 * c)
                finish(2 + 2 * c)
        qk(j, xn, 0)
        ob[j] = pv_mxu(j, *softmax(0))

    nj = 1 + 2 * NCH
    finish(nj)
    for half in range(2):
        finish(nj + 1 + half)
        x = lax.fori_loop(half * 8, half * 8 + 8, lambda j, a: a + out_proj(j, ob[j]), x)
    h = ffn_up(x)
    finish(nj + 3)
    x = ffn_down(x, h)

    xn = layernorm(x)
    nv = NP - N_MXU_PV
    outs, ys = [], []
    for j in range(NP + 1):
        if j < NP:
            qk(j, xn, j)
        if 1 <= j <= nv:
            outs.append(pv_vpu(j - 1, *softmax(j - 1), (j - 1) % 2))
        while len(ys) < (j * 3) // 4 - 1:
            ys.append(out_proj(len(ys), outs[len(ys)]))
    for j in range(nv, NP):
        outs.append(pv_mxu(j, *softmax(j)))
    for j in list(range(nv, NP)) + list(range(len(ys), nv)):
        ys.append(out_proj(j, outs[j]))
    for y in ys:
        x = x + y
    x = ffn_down(x, ffn_up(x))
    o_ref[0] = x[0:1].astype(o_ref.dtype)


@jax.jit
def pallas_interleave_layers__sliding_block_cached__dense_activation_gelu__decode_kernel(
    A_x: jax.Array,
    A_k_cache: jax.Array,
    A_v_cache: jax.Array,
    A_wq: jax.Array,
    A_wo: jax.Array,
    B_x: jax.Array,
    B_w1: jax.Array,
    B_b1: jax.Array,
    B_w2: jax.Array,
    B_b2: jax.Array,
):
    del B_x
    sk = A_k_cache.shape[2]
    kt = _tiles(A_k_cache.transpose(0, 1, 3, 2).reshape(H * DH, sk))
    vt = _tiles(A_v_cache.transpose(0, 1, 3, 2).reshape(H * DH, sk))

    def resident(r, c):
        return pltpu.VMEM((r // 16, c // 128, 16, 128), BF)

    return pl.pallas_call(
        _kernel,
        in_specs=[pl.BlockSpec(memory_space=pl.ANY)] * 9,
        out_specs=pl.BlockSpec(memory_space=pltpu.VMEM),
        out_shape=jax.ShapeDtypeStruct(A_x.shape, A_x.dtype),
        scratch_shapes=[
            resident(H * DH, W), resident(H * DH, W),
            resident(D, H * DH), resident(H * DH, D), resident(D, F), resident(F, D),
            pltpu.VMEM(A_x.shape, BF), pltpu.VMEM((F,), BF), pltpu.VMEM((D,), BF),
            pltpu.VMEM((NP, 8, 384), F32),
            pltpu.VMEM((NP, CT // 4, 12, 8, 128), F32),
            pltpu.VMEM((2, 2, CT, 8, 128), F32),
            pltpu.SemaphoreType.DMA((2 * NCH + 8,)),
        ],
        compiler_params=pltpu.CompilerParams(vmem_limit_bytes=127 * 2**20),
    )(A_x, kt, vt, _tiles(A_wq), _tiles(A_wo), _tiles(B_w1), B_b1, _tiles(B_w2), B_b2)
```

```python
import jax
import jax.numpy as jnp
from jax import lax
import jax.experimental.pallas as pl
import jax.experimental.pallas.tpu as pltpu

D, F = 640, 1536
H, DH = 32, 192
W = 4096
NP = H // 2
CT = W // 128
CHUNKS = (0, 8, 13, 15, 16)

BF, F32, U32 = jnp.bfloat16, jnp.float32, jnp.uint32


def _tiles(a):
    r, c = a.shape
    return a.reshape(r // 16, 2, 8, c // 128, 128).transpose(0, 1, 3, 2, 4)


def _tree(xs, op):
    while len(xs) > 1:
        xs = [op(*xs[i:i + 2]) if i + 1 < len(xs) else xs[i] for i in range(0, len(xs), 2)]
    return xs[0]


def _kernel(x_hbm, k_hbm, v_hbm, wq_hbm, wo_hbm, w1_hbm, b1_hbm, w2_hbm, b2_hbm, o_ref,
            kb, vb, wqb, wob, w1b, w2b, xb, b1b, b2b, ob, sems):
    ct0 = k_hbm.shape[2] - CT
    ku, vu, wqu, wou, w1u, w2u = (r.bitcast(U32) for r in (kb, vb, wqb, wob, w1b, w2b))

    jobs = []

    def job(src, dst, r0, nr, c0):
        jobs.append([pltpu.make_async_copy(src.at[pl.ds(r0, nr), par, pl.ds(c0, dst.shape[1])],
                                           dst.at[pl.ds(r0, nr), :, pl.ds(par * 8, 8), :],
                                           sems.at[len(jobs)]) for par in range(2)])

    job(wq_hbm, wqb, 0, D // 16, 0)
    for a, b in zip(CHUNKS, CHUNKS[1:]):
        job(k_hbm, kb, a * 24, (b - a) * 24, ct0)
        job(v_hbm, vb, a * 24, (b - a) * 24, ct0)
    job(wo_hbm, wob, 0, NP * 24, 0)
    job(w1_hbm, w1b, 0, D // 16, 0)
    job(w2_hbm, w2b, 0, F // 16, 0)
    small = [pltpu.make_async_copy(s, d, sems.at[len(jobs) + i])
             for i, (s, d) in enumerate(((x_hbm, xb), (b1_hbm, b1b), (b2_hbm, b2b)))]

    def start(j):
        for cp in jobs[j]:
            cp.start()

    def finish(j):
        for cp in jobs[j]:
            cp.wait()

    row = lax.broadcasted_iota(jnp.int32, (8, 128), 0)
    lane = lax.broadcasted_iota(jnp.int32, (8, 128), 1)
    even = (row & 1) == 0
    own = (even, even == (lane < 64), ~even)
    quad = [(row >> 1) == u for u in range(4)]

    def wtile(ref, r0, n, c):
        return pltpu.bitcast(ref[pl.ds(r0, n), c].reshape(n * 8, 128), BF)

    def dot(a, b):
        return jnp.dot(a, b, preferred_element_type=F32)

    def project(lhs, ref, r0, n, c0, nc):
        return dot(lhs, jnp.concatenate([wtile(ref, r0, n, c0 + c) for c in range(nc)], axis=1))

    def layernorm(x):
        m = jnp.sum(x, axis=-1, keepdims=True) * (1.0 / D)
        xc = x - m
        v = jnp.sum(xc * xc, axis=-1, keepdims=True) * (1.0 / D)
        return (xc / jnp.sqrt(v + 1e-5)).astype(BF)

    def ffn_up(x):
        h = project(layernorm(x), w1u, 0, D // 16, 0, F // 128) + b1b[...].astype(F32).reshape(1, F)
        return jax.nn.gelu(h, approximate=True).astype(BF)

    def ffn_down(x, h):
        return x + (project(h, w2u, 0, F // 16, 0, D // 128) + b2b[...].astype(F32).reshape(1, D))

    def q_proj(j, xn):
        return project(xn, wqu, 0, D // 16, j * 3, 3)

    def scores(j, q):
        lhs = [[jnp.where(own[t] & quad[u], q[:, t * 128:(t + 1) * 128], 0.0).astype(BF)
                for u in range(4)] for t in range(3)]
        out = []
        for g in range(CT // 4):
            s = None
            for t in range(3):
                for u in range(4):
                    d = dot(lhs[t][u], wtile(ku, j * 24 + t * 8, 8, g * 4 + u))
                    s = d if s is None else s + d
            out.append(s * (DH ** -0.5))
        return out

    def over_head(x, op):
        x = op(x, pltpu.roll(x, 2, 0))
        return op(x, pltpu.roll(x, 4, 0))

    def softmax(s):
        m = jnp.max(over_head(_tree(s, jnp.maximum), jnp.maximum), axis=-1, keepdims=True)
        p = [jnp.exp(x - m) for x in s]
        l = jnp.sum(over_head(_tree(p, jnp.add), jnp.add), axis=-1, keepdims=True)
        return p, 1.0 / l

    def retile_v(j):
        @pl.loop(0, CT // 4)
        def _(g):
            for t in range(3):
                for u in range(4):
                    r0, c = j * 24 + t * 8, g * 4 + u
                    vu[pl.ds(r0, 8), c] = pltpu.bitcast(wtile(vu, r0, 8, c).T, U32).reshape(8, 8, 128)

    def pv(j, p, inv):
        acc = [None] * 3
        for g in range(CT // 4):
            lhs = [jnp.where(quad[u], p[g], 0.0).astype(BF) for u in range(4)]
            for t in range(3):
                for u in range(4):
                    d = dot(lhs[u], wtile(vu, j * 24 + t * 8, 8, g * 4 + u))
                    acc[t] = d if acc[t] is None else acc[t] + d
        out = []
        for t in range(3):
            o = over_head(acc[t], jnp.add) * inv
            out.append(jnp.where(own[t], o, pltpu.roll(o, 1, 0)))
        return jnp.concatenate(out, axis=1)

    def out_proj(j, o):
        return project(o.astype(BF), wou, j * 24, 24, 0, D // 128)

    start(0)
    for cp in small:
        cp.start()
    for j in range(1, len(jobs)):
        start(j)
    for cp in small:
        cp.wait()
    x = jnp.broadcast_to(xb[0].astype(F32), (8, D))
    xn = layernorm(x)
    finish(0)

    @pl.loop(0, NP)
    def _(j):
        for c, first in enumerate(CHUNKS[:-1]):
            @pl.when(j == first)
            def _():
                finish(1 + 2 * c)
                finish(2 + 2 * c)
        retile_v(j)
        ob[j] = pv(j, *softmax(scores(j, q_proj(j, xn))))

    finish(-3)
    x = x + project(jnp.concatenate([ob[j] for j in range(NP)], axis=1).astype(BF), wou, 0, NP * 24, 0, D // 128)
    finish(-2)
    h = ffn_up(x)
    finish(-1)
    x = ffn_down(x, h)

    xn = layernorm(x)
    q, s, o = {}, {}, {}
    for j in range(-1, NP + 2):
        if j + 1 < NP:
            q[j + 1] = q_proj(j + 1, xn)
            if j == -1:
                continue
        if j < NP:
            s[j] = scores(j, q[j])
        if 0 <= j - 1 < NP:
            o[j - 1] = pv(j - 1, *softmax(s[j - 1]))
        if 0 <= j - 2:
            x = x + out_proj(j - 2, o[j - 2])
    x = ffn_down(x, ffn_up(x))
    o_ref[0] = x[0:1].astype(o_ref.dtype)


@jax.jit
def pallas_interleave_layers__sliding_block_cached__dense_activation_gelu__decode_kernel(
    A_x: jax.Array,
    A_k_cache: jax.Array,
    A_v_cache: jax.Array,
    A_wq: jax.Array,
    A_wo: jax.Array,
    B_x: jax.Array,
    B_w1: jax.Array,
    B_b1: jax.Array,
    B_w2: jax.Array,
    B_b2: jax.Array,
):
    del B_x
    sk = A_k_cache.shape[2]
    kt = _tiles(A_k_cache.transpose(0, 1, 3, 2).reshape(H * DH, sk))
    vt = _tiles(A_v_cache.transpose(0, 1, 3, 2).reshape(H * DH, sk))

    def resident(r, c):
        return pltpu.VMEM((r // 16, c // 128, 16, 128), BF)

    return pl.pallas_call(
        _kernel,
        in_specs=[pl.BlockSpec(memory_space=pl.ANY)] * 9,
        out_specs=pl.BlockSpec(memory_space=pltpu.VMEM),
        out_shape=jax.ShapeDtypeStruct(A_x.shape, A_x.dtype),
        scratch_shapes=[
            resident(H * DH, W), resident(H * DH, W),
            resident(D, H * DH), resident(H * DH, D), resident(D, F), resident(F, D),
            pltpu.VMEM(A_x.shape, BF), pltpu.VMEM((F,), BF), pltpu.VMEM((D,), BF),
            pltpu.VMEM((NP, 8, 384), F32),
            pltpu.SemaphoreType.DMA((2 * len(CHUNKS) + 5,)),
        ],
        compiler_params=pltpu.CompilerParams(vmem_limit_bytes=120 * 2**20),
    )(A_x, kt, vt, _tiles(A_wq), _tiles(A_wo), _tiles(B_w1), B_b1, _tiles(B_w2), B_b2)
```

```python
import jax
import jax.numpy as jnp
from jax import lax
import jax.experimental.pallas as pl
import jax.experimental.pallas.tpu as pltpu

D, F = 640, 1536
H, DH = 32, 192
W = 4096
NP = H // 2
CT = W // 128
CHUNKS = (0, 8, 13, 15, 16)
G = 2
SPLIT = (7, 6)
SPLIT_LAST = (7, 0)
PART = 2
A_P, A_INV = 12, 44
B_O, B_END = 96, 320

BF, F32, U32 = jnp.bfloat16, jnp.float32, jnp.uint32


def _tiles(a):
    r, c = a.shape
    return a.reshape(r // 16, 2, 8, c // 128, 128).transpose(0, 1, 3, 2, 4)


def _tree(xs, op):
    while len(xs) > 1:
        xs = [op(*xs[i:i + 2]) if i + 1 < len(xs) else xs[i] for i in range(0, len(xs), 2)]
    return xs[0]


def _kernel(x_hbm, k_hbm, v_hbm, wq_hbm, wo_hbm, w1_hbm, b1_hbm, w2_hbm, b2_hbm, o_ref,
            kb, vb, wqb, wob, w1b, w2b, xb, b1b, b2b, ob, sa, sb, sems):
    ct0 = k_hbm.shape[2] - CT
    ku, vu, wqu, wou, w1u, w2u = (r.bitcast(U32) for r in (kb, vb, wqb, wob, w1b, w2b))

    jobs = []

    def job(src, dst, r0, nr, c0):
        jobs.append([pltpu.make_async_copy(src.at[pl.ds(r0, nr), par, pl.ds(c0, dst.shape[1])],
                                           dst.at[pl.ds(r0, nr), :, pl.ds(par * 8, 8), :],
                                           sems.at[len(jobs)]) for par in range(2)])

    job(wq_hbm, wqb, 0, D // 16, 0)
    for a, b in zip(CHUNKS, CHUNKS[1:]):
        job(k_hbm, kb, a * 24, (b - a) * 24, ct0)
        job(v_hbm, vb, a * 24, (b - a) * 24, ct0)
    job(wo_hbm, wob, 0, NP * 24, 0)
    job(w1_hbm, w1b, 0, D // 16, 0)
    job(w2_hbm, w2b, 0, F // 16, 0)
    small = [pltpu.make_async_copy(s, d, sems.at[len(jobs) + i])
             for i, (s, d) in enumerate(((x_hbm, xb), (b1_hbm, b1b), (b2_hbm, b2b)))]

    def start(j):
        for cp in jobs[j]:
            cp.start()

    def finish(j):
        for cp in jobs[j]:
            cp.wait()

    row = lax.broadcasted_iota(jnp.int32, (8, 128), 0)
    lane = lax.broadcasted_iota(jnp.int32, (8, 128), 1)
    even = (row & 1) == 0
    own = (even, even == (lane < 64), ~even)
    quad = [(row >> 1) == u for u in range(4)]

    def wtile(ref, r0, n, c):
        return pltpu.bitcast(ref[pl.ds(r0, n), c].reshape(n * 8, 128), BF)

    def dot(a, b):
        return jnp.dot(a, b, preferred_element_type=F32)

    def project(lhs, ref, r0, n, c0, nc):
        return dot(lhs, jnp.concatenate([wtile(ref, r0, n, c0 + c) for c in range(nc)], axis=1))

    def layernorm(x):
        m = jnp.sum(x, axis=-1, keepdims=True) * (1.0 / D)
        xc = x - m
        v = jnp.sum(xc * xc, axis=-1, keepdims=True) * (1.0 / D)
        return (xc / jnp.sqrt(v + 1e-5)).astype(BF)

    def ffn_up(x):
        h = project(layernorm(x), w1u, 0, D // 16, 0, F // 128) + b1b[...].astype(F32).reshape(1, F)
        return jax.nn.gelu(h, approximate=True).astype(BF)

    def ffn_down(x, h):
        return x + (project(h, w2u, 0, F // 16, 0, D // 128) + b2b[...].astype(F32).reshape(1, D))

    def q_proj(j, xn):
        return project(xn, wqu, 0, D // 16, j * 3, 3)

    def q_lhs(q):
        return [[jnp.where(own[t] & quad[u], q[:, t * 128:(t + 1) * 128], 0.0)
                 for u in range(4)] for t in range(3)]

    def scores(j, q):
        lhs = [[z.astype(BF) for z in zs] for zs in q_lhs(q)]
        out = []
        for g in range(CT // 4):
            s = None
            for t in range(3):
                for u in range(4):
                    d = dot(lhs[t][u], wtile(ku, j * 24 + t * 8, 8, g * 4 + u))
                    s = d if s is None else s + d
            out.append(s * (DH ** -0.5))
        return out

    def over_head(x, op):
        x = op(x, pltpu.roll(x, 2, 0))
        return op(x, pltpu.roll(x, 4, 0))

    def softmax(s):
        m = jnp.max(over_head(_tree(s, jnp.maximum), jnp.maximum), axis=-1, keepdims=True)
        p = [jnp.exp(x - m) for x in s]
        l = jnp.sum(over_head(_tree(p, jnp.add), jnp.add), axis=-1, keepdims=True)
        return p, jnp.broadcast_to(1.0 / l, (8, 128))

    def retile_v(j, g0):
        @pl.loop(g0, CT // 4)
        def _(g):
            for t in range(3):
                for u in range(4):
                    r0, c = j * 24 + t * 8, g * 4 + u
                    vu[pl.ds(r0, 8), c] = pltpu.bitcast(wtile(vu, r0, 8, c).T, U32).reshape(8, 8, 128)

    def head_rows(acc):
        out = []
        for t in range(3):
            o = over_head(acc[t], jnp.add)
            out.append(jnp.where(own[t], o, pltpu.roll(o, 1, 0)))
        return out

    def normalize(o, inv):
        return jnp.concatenate([o[t] * jnp.where(own[t], inv, pltpu.roll(inv, 1, 0)) for t in range(3)], axis=1)

    def pv(j, p, inv):
        acc = [None] * 3
        for g in range(CT // 4):
            lhs = [jnp.where(quad[u], p[g], 0.0).astype(BF) for u in range(4)]
            for t in range(3):
                for u in range(4):
                    d = lax.dot_general(lhs[u], wtile(vu, j * 24 + t * 8, 8, g * 4 + u),
                                        (((1,), (1,)), ((), ())), preferred_element_type=F32)
                    acc[t] = d if acc[t] is None else acc[t] + d
        return normalize(head_rows(acc), inv)

    def out_proj(j, o):
        return project(o.astype(BF), wou, j * 24, 24, 0, D // 128)

    start(0)
    for cp in small:
        cp.start()
    for j in range(1, len(jobs)):
        start(j)
    for cp in small:
        cp.wait()
    x = jnp.broadcast_to(xb[0].astype(F32), (8, D))
    xn = layernorm(x)
    finish(0)

    @pl.loop(0, NP)
    def _(j):
        for c, first in enumerate(CHUNKS[:-1]):
            @pl.when(j == first)
            def _():
                finish(1 + 2 * c)
                finish(2 + 2 * c)
        ob[j] = pv(j, *softmax(scores(j, q_proj(j, xn))))
        g0 = SPLIT[0]
        for k in range(1, G):
            g0 = jnp.where((j & (G - 1)) == k, SPLIT[k], g0)
        for k in range(G):
            g0 = jnp.where(j == NP - G + k, SPLIT_LAST[k], g0)
        retile_v(j, g0)

    finish(-3)
    x = x + project(jnp.concatenate([ob[j] for j in range(NP)], axis=1).astype(BF), wou, 0, NP * 24, 0, D // 128)
    finish(-2)
    h = ffn_up(x)
    finish(-1)
    x = ffn_down(x, h)

    xn = layernorm(x)

    def operand(v):
        return pltpu.bitcast(jnp.concatenate([v, jnp.zeros_like(v)], axis=0).astype(BF), U32)

    def mxu(lhs, ref, r0, c):
        return dot(pltpu.bitcast(lhs, BF), wtile(ref, r0, 8, c))[:8]

    def parts(g0):
        return [range(a, min(a + PART, g0)) for a in range(0, g0, PART)]

    def bulk(i, split, more):
        for k, g0 in enumerate(split):
            r0 = (i * G + k) * 24
            for e in range(2):
                for n, gs in enumerate(parts(g0)):
                    pu = {}
                    for g in gs:
                        pg = pltpu.bitcast(sa[k, A_P + g * 4], F32)
                        for u in range(4):
                            pu[g, u] = jnp.broadcast_to(pg[2 * u + e:2 * u + e + 1], (16, 128))
                    for r in range(12):
                        acc = _tree([pltpu.bitcast(vu[r0 + e * 12 + r, g * 4 + u], BF).astype(F32) * pu[g, u]
                                     for g in gs for u in range(4)], jnp.add)
                        sb[k, B_O + gs[0] * 48 // PART + e * 24 + 2 * r] = acc[:8]
                        sb[k, B_O + gs[0] * 48 // PART + e * 24 + 2 * r + 1] = acc[8:]
            for g in range(g0, 8):
                for n in range(12):
                    sb[k, B_END - (8 - g) * 12 + n] = mxu(sa[k, A_P + g * 4 + n % 4], vu, r0 + n // 4 * 8, g * 4 + n % 4)
        for k in range(G if more else 0):
            for g in range(8):
                for n in range(12):
                    sb[k, g * 12 + n] = mxu(sa[k, n], ku, ((i + 1) * G + k) * 24 + n // 4 * 8, g * 4 + n % 4)

    def prep_q(i):
        for k in range(G):
            for n, z in enumerate(sum(q_lhs(q_proj(i * G + k, xn)), [])):
                sa[k, n] = operand(z)

    def prep_p(split):
        for k, g0 in enumerate(split):
            p, inv = softmax([_tree([sb[k, g * 12 + n] for n in range(12)], jnp.add) * (DH ** -0.5)
                              for g in range(8)])
            sa[k, A_INV] = pltpu.bitcast(inv, U32)
            for g in range(8):
                if g < g0:
                    sa[k, A_P + g * 4] = pltpu.bitcast(p[g], U32)
                else:
                    for u in range(4):
                        sa[k, A_P + g * 4 + u] = operand(jnp.where(quad[u], p[g], 0.0))

    def gather_o(split):
        for k, g0 in enumerate(split):
            o = head_rows([_tree([sb[k, B_END - (8 - g) * 12 + t * 4 + u] for g in range(g0, 8) for u in range(4)],
                                 jnp.add) for t in range(3)])
            for t in range(3 if g0 else 0):
                a = jnp.concatenate([_tree([sb[k, B_O + gs[0] * 48 // PART + t * 16 + r] for gs in parts(g0)], jnp.add)
                                     for r in range(16)], axis=0).T
                a = _tree([a[r * 8:(r + 1) * 8] for r in range(16)], jnp.add)
                o[t] = o[t] + over_head(a + pltpu.roll(a, 1, 0), jnp.add)
            ob[k] = normalize(o, pltpu.bitcast(sa[k, A_INV], F32))

    def add_out(i, valid):
        y = _tree([out_proj(i * G + k, ob[k]) for k in range(G)], jnp.add)
        for c in range(D // 128):
            ob[G + c, :, 0:128] += jnp.where(valid, y[:, c * 128:(c + 1) * 128], 0.0)

    ns = NP // G
    for c in range(D // 128):
        ob[G + c, :, 0:128] = x[:, c * 128:(c + 1) * 128]
    prep_q(0)
    bulk(-1, (), True)
    prep_q(1)
    prep_p(SPLIT)

    @pl.loop(0, 2 * ns - 1)
    def _(n):
        i = n >> 1

        @pl.when(((n & 1) == 0) & (n < 2 * ns - 2))
        def _():
            bulk(i, SPLIT, True)

        @pl.when(((n & 1) == 1) & (n < 2 * ns - 3))
        def _():
            add_out(jnp.maximum(i - 1, 0), i >= 1)
            prep_q(i + 2)
            gather_o(SPLIT)
            prep_p(SPLIT)

        @pl.when(n == 2 * ns - 3)
        def _():
            add_out(ns - 3, True)
            gather_o(SPLIT)
            prep_p(SPLIT_LAST)

        @pl.when(n == 2 * ns - 2)
        def _():
            bulk(ns - 1, SPLIT_LAST, False)

    add_out(ns - 2, True)
    gather_o(SPLIT_LAST)
    add_out(ns - 1, True)
    x = jnp.concatenate([ob[G + c, :, 0:128] for c in range(D // 128)], axis=1)
    x = ffn_down(x, ffn_up(x))
    o_ref[0] = x[0:1].astype(o_ref.dtype)


@jax.jit
def pallas_interleave_layers__sliding_block_cached__dense_activation_gelu__decode_kernel(
    A_x: jax.Array,
    A_k_cache: jax.Array,
    A_v_cache: jax.Array,
    A_wq: jax.Array,
    A_wo: jax.Array,
    B_x: jax.Array,
    B_w1: jax.Array,
    B_b1: jax.Array,
    B_w2: jax.Array,
    B_b2: jax.Array,
):
    del B_x
    sk = A_k_cache.shape[2]
    kt = _tiles(A_k_cache.transpose(0, 1, 3, 2).reshape(H * DH, sk))
    vt = _tiles(A_v_cache.transpose(0, 1, 3, 2).reshape(H * DH, sk))

    def resident(r, c):
        return pltpu.VMEM((r // 16, c // 128, 16, 128), BF)

    return pl.pallas_call(
        _kernel,
        in_specs=[pl.BlockSpec(memory_space=pl.ANY)] * 9,
        out_specs=pl.BlockSpec(memory_space=pltpu.VMEM),
        out_shape=jax.ShapeDtypeStruct(A_x.shape, A_x.dtype),
        scratch_shapes=[
            resident(H * DH, W), resident(H * DH, W),
            resident(D, H * DH), resident(H * DH, D), resident(D, F), resident(F, D),
            pltpu.VMEM(A_x.shape, BF), pltpu.VMEM((F,), BF), pltpu.VMEM((D,), BF),
            pltpu.VMEM((NP, 8, 384), F32),
            pltpu.VMEM((G, A_INV + 1, 8, 128), U32), pltpu.VMEM((G, B_END, 8, 128), F32),
            pltpu.SemaphoreType.DMA((2 * len(CHUNKS) + 5,)),
        ],
        compiler_params=pltpu.CompilerParams(vmem_limit_bytes=124 * 2**20),
    )(A_x, kt, vt, _tiles(A_wq), _tiles(A_wo), _tiles(B_w1), B_b1, _tiles(B_w2), B_b2)
```

```python
import functools

import jax
import jax.numpy as jnp
from jax import lax
import jax.experimental.pallas as pl
import jax.experimental.pallas.tpu as pltpu

D, F = 640, 1536
H, DH = 32, 192
W = 4096
NP = H // 2
CT = W // 128
CHUNKS = (0, 8, 13, 15, 16)
FS = 1280
STEPS = ((8, 8), (8, 8, 7), (7, 6, 6, 7), (6, 6, 6, 5), (8, 2, 0))
PART = 2
A_P, A_INV = 12, 44
B_O, B_END = 96, 320

BF, F32, U32 = jnp.bfloat16, jnp.float32, jnp.uint32


def _tiles(a):
    r, c = a.shape
    return a.reshape(r // 16, 2, 8, c // 128, 128).transpose(0, 1, 3, 2, 4)


def _tree(xs, op):
    while len(xs) > 1:
        xs = [op(*xs[i:i + 2]) if i + 1 < len(xs) else xs[i] for i in range(0, len(xs), 2)]
    return xs[0]


def _kernel(x_hbm, k_hbm, v_hbm, wq_hbm, wo_hbm, w1_hbm, b1_hbm, w2_hbm, b2_hbm, o_ref,
            kb, vb, wqb, wob, w1b, w2b, xb, b1b, b2b, ob, xs, sa, sb, sems):
    ct0 = k_hbm.shape[2] - CT
    ku, vu, wqu, wou, w1u, w2u = (r.bitcast(U32) for r in (kb, vb, wqb, wob, w1b, w2b))

    jobs = []

    def job(src, dst, r0, nr, c0):
        jobs.append([pltpu.make_async_copy(src.at[pl.ds(r0, nr), par, pl.ds(c0, dst.shape[1])],
                                           dst.at[pl.ds(r0, nr), :, pl.ds(par * 8, 8), :],
                                           sems.at[len(jobs)]) for par in range(2)])

    job(wq_hbm, wqb, 0, D // 16, 0)
    for a, b in zip(CHUNKS, CHUNKS[1:]):
        job(k_hbm, kb, a * 24, (b - a) * 24, ct0)
        job(v_hbm, vb, a * 24, (b - a) * 24, ct0)
    job(wo_hbm, wob, 0, NP * 24, 0)
    job(w1_hbm, w1b, 0, D // 16, 0)
    job(w2_hbm, w2b, 0, FS // 16, 0)
    job(w2_hbm, w2b, FS // 16, (F - FS) // 16, 0)
    small = [pltpu.make_async_copy(s, d, sems.at[len(jobs) + i])
             for i, (s, d) in enumerate(((x_hbm, xb), (b1_hbm, b1b), (b2_hbm, b2b)))]

    def start(j):
        for cp in jobs[j]:
            cp.start()

    def finish(j):
        for cp in jobs[j]:
            cp.wait()

    row = lax.broadcasted_iota(jnp.int32, (8, 128), 0)
    lane = lax.broadcasted_iota(jnp.int32, (8, 128), 1)
    even = (row & 1) == 0
    own = (even, even == (lane < 64), ~even)
    quad = [(row >> 1) == u for u in range(4)]

    def wtile(ref, r0, n, c):
        return pltpu.bitcast(ref[pl.ds(r0, n), c].reshape(n * 8, 128), BF)

    def dot(a, b):
        return jnp.dot(a, b, preferred_element_type=F32)

    def project(lhs, ref, r0, n, c0, nc):
        return dot(lhs, jnp.concatenate([wtile(ref, r0, n, c0 + c) for c in range(nc)], axis=1))

    def layernorm(x):
        m = jnp.sum(x, axis=-1, keepdims=True) * (1.0 / D)
        xc = x - m
        v = jnp.sum(xc * xc, axis=-1, keepdims=True) * (1.0 / D)
        return xc.astype(BF), lax.rsqrt(v + 1e-5)

    def ffn_up(x):
        xc, rstd = layernorm(x)
        h = project(xc, w1u, 0, D // 16, 0, F // 128) * rstd + b1b[...].astype(F32).reshape(1, F)
        return jax.nn.gelu(h, approximate=True).astype(BF)

    def ffn_down(h, a, b):
        return project(h[:, a:b], w2u, a // 16, (b - a) // 16, 0, D // 128)

    def q_proj(j, xn):
        return project(xn[0], wqu, 0, D // 16, j * 3, 3) * xn[1]

    def q_lhs(q):
        return [[jnp.where(own[t] & quad[u], q[:, t * 128:(t + 1) * 128], 0.0)
                 for u in range(4)] for t in range(3)]

    def scores(j, q):
        lhs = [[z.astype(BF) for z in zs] for zs in q_lhs(q)]
        out = []
        for g in range(CT // 4):
            s = None
            for t in range(3):
                for u in range(4):
                    d = dot(lhs[t][u], wtile(ku, j * 24 + t * 8, 8, g * 4 + u))
                    s = d if s is None else s + d
            out.append(s * (DH ** -0.5))
        return out

    def over_head(x, op):
        x = op(x, pltpu.roll(x, 2, 0))
        return op(x, pltpu.roll(x, 4, 0))

    def softmax(s):
        m = jnp.max(over_head(_tree(s, jnp.maximum), jnp.maximum), axis=-1, keepdims=True)
        p = [jnp.exp(x - m) for x in s]
        l = jnp.sum(over_head(_tree(p, jnp.add), jnp.add), axis=-1, keepdims=True)
        return p, jnp.broadcast_to(1.0 / l, (8, 128))

    def retile_v(j, g0):
        @pl.loop(g0, CT // 4)
        def _(g):
            for t in range(3):
                for u in range(4):
                    r0, c = j * 24 + t * 8, g * 4 + u
                    vu[pl.ds(r0, 8), c] = pltpu.bitcast(wtile(vu, r0, 8, c).T, U32).reshape(8, 8, 128)

    def head_rows(acc):
        out = []
        for t in range(3):
            o = over_head(acc[t], jnp.add)
            out.append(jnp.where(own[t], o, pltpu.roll(o, 1, 0)))
        return out

    def normalize(o, inv):
        return jnp.concatenate([o[t] * jnp.where(own[t], inv, pltpu.roll(inv, 1, 0)) for t in range(3)], axis=1)

    def pv(j, p, inv):
        acc = [None] * 3
        for g in range(CT // 4):
            lhs = [jnp.where(quad[u], p[g], 0.0).astype(BF) for u in range(4)]
            for t in range(3):
                for u in range(4):
                    d = lax.dot_general(lhs[u], wtile(vu, j * 24 + t * 8, 8, g * 4 + u),
                                        (((1,), (1,)), ((), ())), preferred_element_type=F32)
                    acc[t] = d if acc[t] is None else acc[t] + d
        return normalize(head_rows(acc), inv)

    def out_proj(j, o):
        return project(o.astype(BF), wou, j * 24, 24, 0, D // 128)

    start(0)
    for cp in small:
        cp.start()
    for j in range(1, len(jobs)):
        start(j)
    for cp in small:
        cp.wait()
    x = jnp.broadcast_to(xb[0].astype(F32), (8, D))
    xn = layernorm(x)
    finish(0)

    @pl.loop(0, NP)
    def _(j):
        for c, first in enumerate(CHUNKS[:-1]):
            @pl.when(j == first)
            def _():
                finish(1 + 2 * c)
                finish(2 + 2 * c)
        ob[j] = pv(j, *softmax(scores(j, q_proj(j, xn))))
        g0 = CT // 4
        for k, split in enumerate(sum(STEPS, ())):
            g0 = jnp.where(j == k, split, g0)
        retile_v(j, g0)

    finish(-4)
    x = x + project(jnp.concatenate([ob[j] for j in range(NP)], axis=1).astype(BF), wou, 0, NP * 24, 0, D // 128)
    finish(-3)
    h = ffn_up(x)
    b2 = b2b[...].astype(F32).reshape(1, D)
    finish(-2)
    x = x + b2 + ffn_down(h, 0, FS)
    finish(-1)
    x = x + ffn_down(h, FS, F)

    xn = layernorm(x)

    def operand(v):
        return pltpu.bitcast(jnp.concatenate([v, jnp.zeros_like(v)], axis=0).astype(BF), U32)

    def mxu(lhs, ref, r0, c):
        return dot(pltpu.bitcast(lhs, BF), wtile(ref, r0, 8, c))[:8]

    def parts(g0):
        return [range(a, min(a + PART, g0)) for a in range(0, g0, PART)]

    def pairs(i):
        if not 0 <= i < len(STEPS):
            return []
        return [(k, sum(map(len, STEPS[:i])) + k, g0) for k, g0 in enumerate(STEPS[i])]

    def bulk(i):
        for k, j, g0 in pairs(i):
            r0 = j * 24
            for e in range(2):
                for n, gs in enumerate(parts(g0)):
                    pu = {}
                    for g in gs:
                        pg = pltpu.bitcast(sa[k, A_P + g * 4], F32)
                        for u in range(4):
                            pu[g, u] = jnp.broadcast_to(pg[2 * u + e:2 * u + e + 1], (16, 128))
                    for r in range(12):
                        acc = _tree([pltpu.bitcast(vu[r0 + e * 12 + r, g * 4 + u], BF).astype(F32) * pu[g, u]
                                     for g in gs for u in range(4)], jnp.add)
                        sb[k, B_O + gs[0] * 48 // PART + e * 24 + 2 * r] = acc[:8]
                        sb[k, B_O + gs[0] * 48 // PART + e * 24 + 2 * r + 1] = acc[8:]
            for g in range(g0, 8):
                for n in range(12):
                    sb[k, B_END - (8 - g) * 12 + n] = mxu(sa[k, A_P + g * 4 + n % 4], vu, r0 + n // 4 * 8, g * 4 + n % 4)
        for k, j, _ in pairs(i + 1):
            for g in range(8):
                for n in range(12):
                    sb[k, g * 12 + n] = mxu(sa[k, n], ku, j * 24 + n // 4 * 8, g * 4 + n % 4)

    def prep_q(i):
        for k, j, _ in pairs(i):
            for n, z in enumerate(sum(q_lhs(q_proj(j, xn)), [])):
                sa[k, n] = operand(z)

    def prep_p(i):
        for k, j, g0 in pairs(i):
            p, inv = softmax([_tree([sb[k, g * 12 + n] for n in range(12)], jnp.add) * (DH ** -0.5)
                              for g in range(8)])
            sa[k, A_INV] = pltpu.bitcast(inv, U32)
            for g in range(8):
                if g < g0:
                    sa[k, A_P + g * 4] = pltpu.bitcast(p[g], U32)
                else:
                    for u in range(4):
                        sa[k, A_P + g * 4 + u] = operand(jnp.where(quad[u], p[g], 0.0))

    def gather_o(i):
        for k, j, g0 in pairs(i):
            o = [0.0] * 3
            if g0 < 8:
                o = head_rows([_tree([sb[k, B_END - (8 - g) * 12 + t * 4 + u]
                                      for g in range(g0, 8) for u in range(4)], jnp.add) for t in range(3)])
            for t in range(3 if g0 else 0):
                a = jnp.concatenate([_tree([sb[k, B_O + gs[0] * 48 // PART + t * 16 + r] for gs in parts(g0)], jnp.add)
                                     for r in range(16)], axis=0).T
                a = _tree([a[r * 8:(r + 1) * 8] for r in range(16)], jnp.add)
                o[t] = o[t] + over_head(a + pltpu.roll(a, 1, 0), jnp.add)
            ob[j] = normalize(o, pltpu.bitcast(sa[k, A_INV], F32))

    def add_out(i):
        for _, j, _ in pairs(i):
            xs[...] += out_proj(j, ob[j])

    def glue(i):
        add_out(i - 1)
        prep_q(i + 2)
        gather_o(i)
        prep_p(i + 1)

    xs[...] = x
    prep_q(0)
    bulk(-1)
    glue(-1)

    @pl.loop(0, 2 * len(STEPS) - 1)
    def _(n):
        for m in range(2 * len(STEPS) - 1):
            pl.when(n == m)(functools.partial((bulk, glue)[m % 2], m // 2))

    glue(len(STEPS) - 1)
    add_out(len(STEPS) - 1)
    x = xs[...]
    x = x + b2 + ffn_down(ffn_up(x), 0, F)
    o_ref[0] = x[0:1].astype(o_ref.dtype)


@jax.jit
def pallas_interleave_layers__sliding_block_cached__dense_activation_gelu__decode_kernel(
    A_x: jax.Array,
    A_k_cache: jax.Array,
    A_v_cache: jax.Array,
    A_wq: jax.Array,
    A_wo: jax.Array,
    B_x: jax.Array,
    B_w1: jax.Array,
    B_b1: jax.Array,
    B_w2: jax.Array,
    B_b2: jax.Array,
):
    del B_x
    sk = A_k_cache.shape[2]
    kt = _tiles(A_k_cache.transpose(0, 1, 3, 2).reshape(H * DH, sk))
    vt = _tiles(A_v_cache.transpose(0, 1, 3, 2).reshape(H * DH, sk))

    slots = max(map(len, STEPS))

    def resident(r, c):
        return pltpu.VMEM((r // 16, c // 128, 16, 128), BF)

    return pl.pallas_call(
        _kernel,
        in_specs=[pl.BlockSpec(memory_space=pl.ANY)] * 9,
        out_specs=pl.BlockSpec(memory_space=pltpu.VMEM),
        out_shape=jax.ShapeDtypeStruct(A_x.shape, A_x.dtype),
        scratch_shapes=[
            resident(H * DH, W), resident(H * DH, W),
            resident(D, H * DH), resident(H * DH, D), resident(D, F), resident(F, D),
            pltpu.VMEM(A_x.shape, BF), pltpu.VMEM((F,), BF), pltpu.VMEM((D,), BF),
            pltpu.VMEM((NP, 8, 384), F32),
            pltpu.VMEM((8, D), F32),
            pltpu.VMEM((slots, A_INV + 1, 8, 128), U32), pltpu.VMEM((slots, B_END, 8, 128), F32),
            pltpu.SemaphoreType.DMA((2 * len(CHUNKS) + 6,)),
        ],
        compiler_params=pltpu.CompilerParams(vmem_limit_bytes=124 * 2**20),
    )(A_x, kt, vt, _tiles(A_wq), _tiles(A_wo), _tiles(B_w1), B_b1, _tiles(B_w2), B_b2)
```

```python
import functools

import jax
import jax.numpy as jnp
from jax import lax
import jax.experimental.pallas as pl
import jax.experimental.pallas.tpu as pltpu

D, F = 640, 1536
H, DH = 32, 192
W = 4096
NP = H // 2
CT = W // 128
CHUNKS = (0, 8, 13, 15, 16)
FS = 1280
STEPS = ((8, 8), (8, 8, 7), (7, 6, 6, 7), (6, 6, 6, 5), (8, 2, 0))
PART = 2
A_P, A_INV = 12, 44
B_O, B_END = 96, 320

BF, F32, U32 = jnp.bfloat16, jnp.float32, jnp.uint32


def _tiles(a):
    r, c = a.shape
    return a.reshape(r // 16, 2, 8, c // 128, 128).transpose(0, 1, 3, 2, 4)


def _words(ref):
    return ref.bitcast(U32)


def _tree(xs, op):
    while len(xs) > 1:
        xs = [op(*xs[i:i + 2]) if i + 1 < len(xs) else xs[i] for i in range(0, len(xs), 2)]
    return xs[0]


def _kernel(x_hbm, k_hbm, v_hbm, wq_hbm, wo_hbm, w1_hbm, b1_hbm, w2_hbm, b2_hbm, o_ref,
            kb, vb, wqb, wob, w1b, w2b, xb, b1b, b2b, ob, xs, sa, sb, sems):
    ct0 = k_hbm.shape[2] - CT
    jobs = []

    def job(src, dst, r0, nr, c0):
        jobs.append([pltpu.make_async_copy(src.at[pl.ds(r0, nr), par, pl.ds(c0, dst.shape[1])],
                                           dst.at[pl.ds(r0, nr), :, pl.ds(par * 8, 8), :],
                                           sems.at[len(jobs)]) for par in range(2)])

    job(wq_hbm, wqb, 0, D // 16, 0)
    for a, b in zip(CHUNKS, CHUNKS[1:]):
        job(k_hbm, kb, a * 24, (b - a) * 24, ct0)
        job(v_hbm, vb, a * 24, (b - a) * 24, ct0)
    job(wo_hbm, wob, 0, NP * 24, 0)
    job(w1_hbm, w1b, 0, D // 16, 0)
    job(w2_hbm, w2b, 0, FS // 16, 0)
    job(w2_hbm, w2b, FS // 16, (F - FS) // 16, 0)
    small = [pltpu.make_async_copy(s, d, sems.at[len(jobs) + i])
             for i, (s, d) in enumerate(((x_hbm, xb), (b1_hbm, b1b), (b2_hbm, b2b)))]

    def start(j):
        for cp in jobs[j]:
            cp.start()

    def finish(j):
        for cp in jobs[j]:
            cp.wait()

    row = lax.broadcasted_iota(jnp.int32, (8, 128), 0)
    lane = lax.broadcasted_iota(jnp.int32, (8, 128), 1)
    even = (row & 1) == 0
    own = (even, even == (lane < 64), ~even)
    quad = [(row >> 1) == u for u in range(4)]

    def wtile(ref, r0, n, c):
        w = ref[pl.ds(r0, n), c].reshape(-1, 128)
        return w if w.dtype == BF else pltpu.bitcast(w, BF)

    def dot(a, b):
        return jnp.dot(a, b, preferred_element_type=F32)

    def project(lhs, ref, r0, n, c0, nc):
        return dot(lhs, jnp.concatenate([wtile(ref, r0, n, c0 + c) for c in range(nc)], axis=1))

    def layernorm(x):
        m = jnp.sum(x, axis=-1, keepdims=True) * (1.0 / D)
        xc = x - m
        v = jnp.sum(xc * xc, axis=-1, keepdims=True) * (1.0 / D)
        return xc.astype(BF), lax.rsqrt(v + 1e-5)

    def ffn_up(x, w1):
        xc, rstd = layernorm(x)
        h = project(xc, w1, 0, D // 16, 0, F // 128) * rstd + b1b[...].astype(F32).reshape(1, F)
        return jax.nn.gelu(h, approximate=True).astype(BF)

    def ffn_down(h, w2, a, b):
        return project(h[:, a:b], w2, a // 16, (b - a) // 16, 0, D // 128)

    def q_proj(j, xn, wq):
        return project(xn[0], wq, 0, D // 16, j * 3, 3) * xn[1]

    def q_lhs(q):
        return [[jnp.where(own[t] & quad[u], q[:, t * 128:(t + 1) * 128], 0.0)
                 for u in range(4)] for t in range(3)]

    def scores(j, q):
        lhs = [[z.astype(BF) for z in zs] for zs in q_lhs(q)]
        out = []
        for g in range(CT // 4):
            s = None
            for t in range(3):
                for u in range(4):
                    d = dot(lhs[t][u], wtile(kb, j * 24 + t * 8, 8, g * 4 + u))
                    s = d if s is None else s + d
            out.append(s * (DH ** -0.5))
        return out

    def over_head(x, op):
        x = op(x, pltpu.roll(x, 2, 0))
        return op(x, pltpu.roll(x, 4, 0))

    def softmax(s):
        m = jnp.max(over_head(_tree(s, jnp.maximum), jnp.maximum), axis=-1, keepdims=True)
        p = [jnp.exp(x - m) for x in s]
        l = jnp.sum(over_head(_tree(p, jnp.add), jnp.add), axis=-1, keepdims=True)
        return p, jnp.broadcast_to(1.0 / l, (8, 128))

    def retile_v(j, g0):
        @pl.loop(g0, CT // 4)
        def _(g):
            for t in range(3):
                for u in range(4):
                    r0, c = j * 24 + t * 8, g * 4 + u
                    vb[pl.ds(r0, 8), c] = wtile(vb, r0, 8, c).T.reshape(8, 16, 128)

    def head_rows(acc):
        out = []
        for t in range(3):
            o = over_head(acc[t], jnp.add)
            out.append(jnp.where(own[t], o, pltpu.roll(o, 1, 0)))
        return out

    def normalize(o, inv):
        return jnp.concatenate([o[t] * jnp.where(own[t], inv, pltpu.roll(inv, 1, 0)) for t in range(3)], axis=1)

    def pv(j, p, inv):
        acc = [None] * 3
        for g in range(CT // 4):
            lhs = [jnp.where(quad[u], p[g], 0.0).astype(BF) for u in range(4)]
            for t in range(3):
                for u in range(4):
                    d = lax.dot_general(lhs[u], wtile(vb, j * 24 + t * 8, 8, g * 4 + u),
                                        (((1,), (1,)), ((), ())), preferred_element_type=F32)
                    acc[t] = d if acc[t] is None else acc[t] + d
        return normalize(head_rows(acc), inv)

    start(0)
    for cp in small:
        cp.start()
    for j in range(1, len(jobs)):
        start(j)
    for cp in small:
        cp.wait()
    x = jnp.broadcast_to(xb[0].astype(F32), (8, D))
    xn = layernorm(x)
    finish(0)

    @pl.loop(0, NP)
    def _(j):
        for c, first in enumerate(CHUNKS[:-1]):
            @pl.when(j == first)
            def _():
                finish(1 + 2 * c)
                finish(2 + 2 * c)
        ob[j] = pv(j, *softmax(scores(j, q_proj(j, xn, wqb))))
        g0 = CT // 4
        for k, split in enumerate(sum(STEPS, ())):
            g0 = jnp.where(j == k, split, g0)
        retile_v(j, g0)

    finish(-4)
    x = x + project(jnp.concatenate([ob[j] for j in range(NP)], axis=1).astype(BF), wob, 0, NP * 24, 0, D // 128)
    finish(-3)
    h = ffn_up(x, w1b)
    b2 = b2b[...].astype(F32).reshape(1, D)
    finish(-2)
    x = x + b2 + ffn_down(h, w2b, 0, FS)
    finish(-1)
    ku, vu, wqu, wou, w1u, w2u = map(_words, (kb, vb, wqb, wob, w1b, w2b))
    x = x + ffn_down(h, w2u, FS, F)

    xn = layernorm(x)

    def operand(v):
        return pltpu.bitcast(jnp.concatenate([v, jnp.zeros_like(v)], axis=0).astype(BF), U32)

    def mxu(lhs, ref, r0, c):
        return dot(pltpu.bitcast(lhs, BF), wtile(ref, r0, 8, c))[:8]

    def parts(g0):
        return [range(a, min(a + PART, g0)) for a in range(0, g0, PART)]

    def pairs(i):
        if not 0 <= i < len(STEPS):
            return []
        return [(k, sum(map(len, STEPS[:i])) + k, g0) for k, g0 in enumerate(STEPS[i])]

    def bulk(i):
        for k, j, g0 in pairs(i):
            r0 = j * 24
            for e in range(2):
                for gs in parts(g0):
                    pu = {}
                    for g in gs:
                        pg = pltpu.bitcast(sa[k, A_P + g * 4], F32)
                        for u in range(4):
                            pu[g, u] = jnp.broadcast_to(pg[2 * u + e:2 * u + e + 1], (16, 128))
                    for r in range(12):
                        acc = _tree([wtile(vu, r0 + e * 12 + r, 1, g * 4 + u).astype(F32) * pu[g, u]
                                     for g in gs for u in range(4)], jnp.add)
                        sb[k, B_O + gs[0] * 48 // PART + e * 24 + 2 * r] = acc[:8]
                        sb[k, B_O + gs[0] * 48 // PART + e * 24 + 2 * r + 1] = acc[8:]
            for g in range(g0, 8):
                for n in range(12):
                    sb[k, B_END - (8 - g) * 12 + n] = mxu(sa[k, A_P + g * 4 + n % 4], vu, r0 + n // 4 * 8, g * 4 + n % 4)
        for k, j, _ in pairs(i + 1):
            for g in range(8):
                for n in range(12):
                    sb[k, g * 12 + n] = mxu(sa[k, n], ku, j * 24 + n // 4 * 8, g * 4 + n % 4)

    def prep_q(i):
        for k, j, _ in pairs(i):
            for n, z in enumerate(sum(q_lhs(q_proj(j, xn, wqu)), [])):
                sa[k, n] = operand(z)

    def prep_p(i):
        for k, j, g0 in pairs(i):
            p, inv = softmax([_tree([sb[k, g * 12 + n] for n in range(12)], jnp.add) * (DH ** -0.5)
                              for g in range(8)])
            sa[k, A_INV] = pltpu.bitcast(inv, U32)
            for g in range(8):
                if g < g0:
                    sa[k, A_P + g * 4] = pltpu.bitcast(p[g], U32)
                else:
                    for u in range(4):
                        sa[k, A_P + g * 4 + u] = operand(jnp.where(quad[u], p[g], 0.0))

    def gather_o(i):
        for k, j, g0 in pairs(i):
            o = [0.0] * 3
            if g0 < 8:
                o = head_rows([_tree([sb[k, B_END - (8 - g) * 12 + t * 4 + u]
                                      for g in range(g0, 8) for u in range(4)], jnp.add) for t in range(3)])
            for t in range(3 if g0 else 0):
                a = jnp.concatenate([_tree([sb[k, B_O + gs[0] * 48 // PART + t * 16 + r] for gs in parts(g0)], jnp.add)
                                     for r in range(16)], axis=0).T
                a = _tree([a[r * 8:(r + 1) * 8] for r in range(16)], jnp.add)
                o[t] = o[t] + over_head(a + pltpu.roll(a, 1, 0), jnp.add)
            ob[j] = normalize(o, pltpu.bitcast(sa[k, A_INV], F32))

    def add_out(i):
        for _, j, _ in pairs(i):
            xs[...] += project(ob[j].astype(BF), wou, j * 24, 24, 0, D // 128)

    def glue(i):
        add_out(i - 1)
        prep_q(i + 2)
        gather_o(i)
        prep_p(i + 1)

    xs[...] = x
    prep_q(0)
    bulk(-1)
    glue(-1)

    @pl.loop(0, 2 * len(STEPS) - 1)
    def _(n):
        for m in range(2 * len(STEPS) - 1):
            pl.when(n == m)(functools.partial((bulk, glue)[m % 2], m // 2))

    glue(len(STEPS) - 1)
    add_out(len(STEPS) - 1)
    x = xs[...]
    x = x + b2 + ffn_down(ffn_up(x, w1u), w2u, 0, F)
    o_ref[0] = x[0:1].astype(o_ref.dtype)


@jax.jit
def pallas_interleave_layers__sliding_block_cached__dense_activation_gelu__decode_kernel(
    A_x: jax.Array,
    A_k_cache: jax.Array,
    A_v_cache: jax.Array,
    A_wq: jax.Array,
    A_wo: jax.Array,
    B_x: jax.Array,
    B_w1: jax.Array,
    B_b1: jax.Array,
    B_w2: jax.Array,
    B_b2: jax.Array,
):
    del B_x
    sk = A_k_cache.shape[2]
    kt = _tiles(A_k_cache.transpose(0, 1, 3, 2).reshape(H * DH, sk))
    vt = _tiles(A_v_cache.transpose(0, 1, 3, 2).reshape(H * DH, sk))

    slots = max(map(len, STEPS))

    def resident(r, c):
        return pltpu.VMEM((r // 16, c // 128, 16, 128), BF)

    return pl.pallas_call(
        _kernel,
        in_specs=[pl.BlockSpec(memory_space=pl.ANY)] * 9,
        out_specs=pl.BlockSpec(memory_space=pltpu.VMEM),
        out_shape=jax.ShapeDtypeStruct(A_x.shape, A_x.dtype),
        scratch_shapes=[
            resident(H * DH, W), resident(H * DH, W),
            resident(D, H * DH), resident(H * DH, D), resident(D, F), resident(F, D),
            pltpu.VMEM(A_x.shape, BF), pltpu.VMEM((F,), BF), pltpu.VMEM((D,), BF),
            pltpu.VMEM((NP, 8, 384), F32),
            pltpu.VMEM((8, D), F32),
            pltpu.VMEM((slots, A_INV + 1, 8, 128), U32), pltpu.VMEM((slots, B_END, 8, 128), F32),
            pltpu.SemaphoreType.DMA((2 * len(CHUNKS) + 6,)),
        ],
        compiler_params=pltpu.CompilerParams(vmem_limit_bytes=124 * 2**20),
    )(A_x, kt, vt, _tiles(A_wq), _tiles(A_wo), _tiles(B_w1), B_b1, _tiles(B_w2), B_b2)
```
